```python
import os as _os
_os.environ.setdefault("JAX_PLATFORMS", "cpu")
import jax
import jax.numpy as jnp

def _softmax(x, axis=-1):
    return jax.nn.softmax(x, axis=axis)
def _gelu(x):
    return jax.nn.gelu(x, approximate=True)
def _silu(x):
    return jax.nn.silu(x)
def _sigmoid(x):
    return jax.nn.sigmoid(x)
def _layernorm(x, axis=-1, eps=1e-5):
    m = jnp.mean(x, axis=axis, keepdims=True)
    v = jnp.var(x, axis=axis, keepdims=True)
    return (x - m) / jnp.sqrt(v + eps)
def _scatter_add(tgt, idx, src, axis=0):
    return tgt.at[idx].add(src)
def _segment_sum(src, seg, n):
    return jax.ops.segment_sum(src, seg, n)
class _Rng:
    def __init__(self, key):
        self._k = key
    def _next(self):
        self._k, sub = jax.random.split(self._k)
        return sub
    def normal(self, shape):
        return jax.random.normal(self._next(), shape, dtype=jnp.bfloat16)
    def randint(self, lo, hi, shape):
        return jax.random.randint(self._next(), shape, lo, hi, dtype=jnp.int32)
    def uniform(self, shape, lo=0.0, hi=1.0):
        return jax.random.uniform(self._next(), shape, jnp.bfloat16, lo, hi)
    def permutation(self, n):
        return jax.random.permutation(self._next(), n)


kernel_name = 'interleave_layers__linear_attn_block__mha_block__prompt'

def setup_inputs():
    _rng = _Rng(jax.random.key(int.from_bytes(__import__("os").urandom(4), "little")))
    _w = (lambda a: (lambda t: t.astype(jnp.bfloat16) if jnp.issubdtype(t.dtype, jnp.floating) else t)(jnp.asarray(a)))
    def _A_setup():
        B, S, D = 1, 2048, 1024
        return {
            "x": _w((lambda *s: _rng.normal(s) * 0.05)(B, S, D)),
            "wqkv": _w((lambda *s: _rng.normal(s) * 0.1)(D, 3 * D)),
            "wo": _w((lambda *s: _rng.normal(s) * 0.1)(D, D)),
        }
    _A_in = _A_setup()

    def _B_setup():
        B, S, D, H = 1, 2048, 1024, 32
        return {
            "x": _w((lambda *s: _rng.normal(s) * 0.05)(B, S, D)),
            "wqkv": _w((lambda *s: _rng.normal(s) * 0.1)(D, 3 * D)),
            "wo": _w((lambda *s: _rng.normal(s) * 0.05)(D, D)),
        }
    _B_in = _B_setup()

    return {
        "A_x": _A_in["x"],
        "A_wqkv": _A_in["wqkv"],
        "A_wo": _A_in["wo"],
        "B_x": _B_in["x"],
        "B_wqkv": _B_in["wqkv"],
        "B_wo": _B_in["wo"],
    }

def reference(A_x, A_wqkv, A_wo, B_x, B_wqkv, B_wo):
    def _A_ref(x, wqkv, wo):
        B, S, D = x.shape
        H = 32; Dh = D // H
        qkv = (lambda x, *d: x.transpose(*d))((x @ wqkv).reshape(B, S, 3, H, Dh), 2, 0, 3, 1, 4)
        q, k, v = qkv[0], qkv[1], qkv[2]
        phi = lambda t: jnp.where(t > 0, t + 1, jnp.exp(t)) + 1e-6
        pq, pk = phi(q), phi(k)
        kv = jnp.einsum("bhsd,bhse->bhde", pk, v)
        z = jnp.einsum("bhsd->bhd", pk)
        num = jnp.einsum("bhqd,bhde->bhqe", pq, kv)
        den = jnp.einsum("bhqd,bhd->bhq", pq, z)[..., None] + 1e-6
        o = num / den
        return (lambda x, *d: x.transpose(*d))(o, 0, 2, 1, 3).reshape(B, S, D) @ wo

    def _B_ref(x, wqkv, wo):
        B, S, D = x.shape
        H = 32
        Dh = D // H
        qkv = (lambda x, *d: x.transpose(*d))((x @ wqkv).reshape(B, S, 3, H, Dh), 2, 0, 3, 1, 4)
        q, k, v = qkv[0], qkv[1], qkv[2]
        scores = jnp.einsum("bhqd,bhkd->bhqk", q, k) * (Dh ** -0.5)
        p = _softmax(scores, axis=-1)
        o = jnp.einsum("bhqk,bhkd->bhqd", p, v)
        return (lambda x, *d: x.transpose(*d))(o, 0, 2, 1, 3).reshape(B, S, D) @ wo

    x = A_x
    x = x + _A_ref(_layernorm(x, axis=-1), A_wqkv, A_wo)
    x = x + _B_ref(_layernorm(x, axis=-1), B_wqkv, B_wo)
    x = x + _A_ref(_layernorm(x, axis=-1), A_wqkv, A_wo)
    x = x + _B_ref(_layernorm(x, axis=-1), B_wqkv, B_wo)
    return x
```

```python
import functools
import math

import jax
import jax.numpy as jnp
from jax import lax
import jax.experimental.pallas as pl
import jax.experimental.pallas.tpu as pltpu

S = 2048
D = 1024
H = 32
DH = D // H
G = D // 128
SB = 128
NSB = 2
TM = SB * NSB
NTM = S // TM
NC = 256
TQ = 128
KC = 128
NKC = S // KC
LA = 2
NWCH = 12
WCH = 3 * D // NWCH

F32 = jnp.float32
BF16 = jnp.bfloat16
Q_SCALE = (DH ** -0.5) * math.log2(math.e)


def _dot(a, b):
    return jnp.dot(a, b, preferred_element_type=F32)


def _dot_nt(a, b):
    return lax.dot_general(a, b, (((1,), (1,)), ((), ())), preferred_element_type=F32)


def _layernorm_bf16(x):
    m = jnp.mean(x, axis=-1, keepdims=True)
    xc = x - m
    v = jnp.mean(xc * xc, axis=-1, keepdims=True)
    return (xc * lax.rsqrt(v + 1e-5)).astype(BF16)


def _phi(t):
    return jnp.where(t > 0, t + 1.0, jnp.exp(t)) + 1e-6


def _rev_rowsum(p):
    n = p.shape[0]
    acc = None
    for t0 in range(0, n, 16):
        for i in range(t0 + 14, t0 - 1, -2):
            t = p[i] + p[i + 1]
            acc = t if acc is None else acc + t
    return acc


def _kernel(x_hbm, wqkva_hbm, woa_hbm, wqkvb_hbm, wob_hbm, out_hbm,
            xio_s, wqkva_s, woa_s, wqkvb_s, wob_s,
            x_s, pq_s, q_s, k_s, vt_s, o_s, kv_s, z_s, kvz_s, sc_s,
            xsem, wsem, osem):

    def x_copy(i):
        rows = pl.ds(pl.multiple_of(i * TM, TM), TM)
        return pltpu.make_async_copy(x_hbm.at[rows, :], xio_s.at[rows, :], xsem.at[i])

    def out_copy(i):
        rows = pl.ds(pl.multiple_of(i * TM, TM), TM)
        return pltpu.make_async_copy(xio_s.at[rows, :], out_hbm.at[rows, :], osem.at[i])

    def wa_copy(j):
        cols = pl.ds(j * WCH, WCH)
        return pltpu.make_async_copy(wqkva_hbm.at[:, cols], wqkva_s.at[:, cols], wsem.at[j])

    woa_copy = pltpu.make_async_copy(woa_hbm, woa_s, wsem.at[NWCH])
    wqkvb_copy = pltpu.make_async_copy(wqkvb_hbm, wqkvb_s, wsem.at[NWCH + 1])
    wob_copy = pltpu.make_async_copy(wob_hbm, wob_s, wsem.at[NWCH + 2])

    a_cols = list(range(D, 3 * D, NC)) + list(range(0, D, NC))

    x_copy(0).start()
    for c0 in a_cols:
        if c0 % WCH == 0:
            wa_copy(c0 // WCH).start()
    for i in range(1, NTM):
        x_copy(i).start()
    woa_copy.start()
    wqkvb_copy.start()
    wob_copy.start()

    def sub_rows(i, sb):
        return pl.ds(pl.multiple_of(i * TM + sb * SB, SB), SB)

    def lin_pass1(i, xns, wait_weights=False):
        pkt = [[None] * G for _ in range(NSB)]
        vb = [[None] * G for _ in range(NSB)]
        for sb in range(NSB):
            rows = sub_rows(i, sb)
            for c0 in a_cols:
                if wait_weights and sb == 0 and c0 % WCH == 0:
                    wa_copy(c0 // WCH).wait()
                r = _dot(xns[sb], wqkva_s[:, c0:c0 + NC])
                if c0 < D:
                    pq_s[rows, c0:c0 + NC] = _phi(r).astype(BF16)
                elif c0 < 2 * D:
                    pk = _phi(r)
                    cz = c0 - D
                    z_s[:, cz:cz + NC] += jnp.sum(pk.reshape(SB // 8, 8, NC), axis=0)
                    for u in range(NC // 128):
                        pkt[sb][cz // 128 + u] = pk[:, u * 128:(u + 1) * 128].T.astype(BF16)
                else:
                    cz = c0 - 2 * D
                    for u in range(NC // 128):
                        vb[sb][cz // 128 + u] = r[:, u * 128:(u + 1) * 128].astype(BF16)
        for g in range(G):
            a = jnp.concatenate([pkt[sb][g] for sb in range(NSB)], axis=1)
            b = jnp.concatenate([vb[sb][g] for sb in range(NSB)], axis=0)
            kv_s[g] += _dot(a, b)

    def lin_reset():
        kv_s[...] = jnp.zeros(kv_s.shape, F32)
        z_s[...] = jnp.zeros(z_s.shape, F32)

    def lin_finalize():
        r = lax.broadcasted_iota(jnp.int32, (128, 128), 0) // DH
        c = lax.broadcasted_iota(jnp.int32, (128, 128), 1) // DH
        same = r == c
        z = jnp.sum(z_s[...], axis=0, keepdims=True)
        for g in range(G):
            zc = jnp.broadcast_to(z[:, g * 128:(g + 1) * 128], (128, 128)).T
            kvz_s[g, :, 0:128] = jnp.where(same, kv_s[g], 0.0).astype(BF16)
            kvz_s[g, :, 128:256] = jnp.where(same, zc, 0.0).astype(BF16)

    def out_proj(rows, a, w_ref):
        parts = []
        for c0 in range(0, D, NC):
            xn = x_s[rows, c0:c0 + NC] + _dot(a, w_ref[:, c0:c0 + NC])
            x_s[rows, c0:c0 + NC] = xn
            parts.append(xn)
        return jnp.concatenate(parts, axis=1)

    def p1_block(i, first):
        x_copy(i).wait()
        xns = []
        for sb in range(NSB):
            rows = sub_rows(i, sb)
            xf = xio_s[rows, :].astype(F32)
            x_s[rows, :] = xf
            xns.append(_layernorm_bf16(xf))
        lin_pass1(i, xns, wait_weights=first)

    lin_reset()
    p1_block(0, True)

    def p1_body(i, c):
        p1_block(i, False)
        return c

    lax.fori_loop(1, NTM, p1_body, 0)

    def p2_body(i, c):
        os_ = []
        for sb in range(NSB):
            rows = sub_rows(i, sb)
            parts = []
            for g in range(G):
                nd = _dot(pq_s[rows, g * 128:(g + 1) * 128], kvz_s[g])
                parts.append((nd[:, :128] / (nd[:, 128:] + 1e-6)).astype(BF16))
            os_.append(jnp.concatenate(parts, axis=1))
        xs = [out_proj(sub_rows(i, sb), os_[sb], woa_s) for sb in range(NSB)]
        for sb in range(NSB):
            rows = sub_rows(i, sb)
            xn = _layernorm_bf16(xs[sb])
            for c0 in list(range(2 * D, 3 * D, NC)) + list(range(0, 2 * D, NC)):
                r = _dot(xn, wqkvb_s[:, c0:c0 + NC])
                if c0 < D:
                    q_s[rows, c0:c0 + NC] = (r * Q_SCALE).astype(BF16)
                elif c0 < 2 * D:
                    k_s[rows, c0 - D:c0 - D + NC] = r.astype(BF16)
                else:
                    cz = c0 - 2 * D
                    blk = i * NSB + sb
                    for u in range(NC // 128):
                        vt_s[blk, cz + u * 128:cz + (u + 1) * 128, :] = (
                            r[:, u * 128:(u + 1) * 128].T.astype(BF16))
        return c

    lane_head = lax.broadcasted_iota(jnp.int32, (TQ, 128), 1) // DH

    def make_qz(qb, g):
        rows = pl.ds(pl.multiple_of(qb * TQ, TQ), TQ)
        qf = q_s[rows, g * 128:(g + 1) * 128].astype(F32)
        parts = [jnp.where(lane_head == j, qf, 0.0) for j in range(4)]
        return jnp.concatenate(parts, axis=0).astype(BF16)

    def qk_chunk(qz, g, c):
        return _dot_nt(k_s[c * KC:(c + 1) * KC, g * 128:(g + 1) * 128], qz)

    def attn_prologue():
        qz = make_qz(0, 0)
        for c in range(LA):
            sc_s[c] = qk_chunk(qz, 0, c)

    def p3_body(qb, carry):
        N = 4 * TQ
        qb_next = jnp.minimum(qb + 1, S // TQ - 1)
        qzs = [make_qz(qb, g) for g in range(G)] + [make_qz(qb_next, 0)]
        pend = {c: sc_s[c] for c in range(LA)}
        rows = pl.ds(pl.multiple_of(qb * TQ, TQ), TQ)
        for g in range(G):
            m = None
            lacc = None
            oacc = [None] * 4
            for c in range(NKC):
                t = g * NKC + c
                tn = t + LA
                sn = qk_chunk(qzs[tn // NKC], (tn // NKC) % G, tn % NKC)
                if tn >= G * NKC:
                    sc_s[tn - G * NKC] = sn
                else:
                    pend[tn] = sn
                s = pend.pop(t).reshape(KC // 8, 8, N)
                mx = jnp.max(s, axis=0)
                if m is not None:
                    mx = jnp.maximum(mx, m)
                mnew = jnp.broadcast_to(jnp.max(mx, axis=0, keepdims=True), (8, N))
                p = jnp.exp2(s - mnew[None])
                ls = _rev_rowsum(p)
                if m is not None:
                    alpha = jnp.exp2(m - mnew)
                    lacc = lacc * alpha + ls
                else:
                    lacc = ls
                p = p.reshape(KC, N)
                for j in range(4):
                    r0 = g * 128 + j * DH
                    vt = vt_s[c, r0:r0 + DH, :]
                    r = _dot(vt, p[:, j * TQ:(j + 1) * TQ].astype(BF16))
                    if m is None:
                        oacc[j] = r
                    else:
                        a = alpha[:, j * TQ:(j + 1) * TQ]
                        oacc[j] = (oacc[j].reshape(DH // 8, 8, TQ) * a[None]).reshape(DH, TQ) + r
                m = mnew
            inv = 1.0 / jnp.sum(lacc, axis=0, keepdims=True)
            ot = jnp.concatenate(
                [oacc[j] * inv[:, j * TQ:(j + 1) * TQ] for j in range(4)], axis=0)
            o_s[rows, g * 128:(g + 1) * 128] = ot.T.astype(BF16)
        return carry

    def p4a_body(i, c):
        xs = [out_proj(sub_rows(i, sb), o_s[sub_rows(i, sb), :], wob_s) for sb in range(NSB)]
        lin_pass1(i, [_layernorm_bf16(x) for x in xs])
        return c

    def p4b_body(i, c):
        for sb in range(NSB):
            rows = sub_rows(i, sb)
            a = o_s[rows, :]
            for c0 in range(0, D, NC):
                xio_s[rows, c0:c0 + NC] = (
                    x_s[rows, c0:c0 + NC] + _dot(a, wob_s[:, c0:c0 + NC])).astype(BF16)
        out_copy(i).start()
        return c

    woa_copy.wait()
    wqkvb_copy.wait()
    wob_copy.wait()

    def rep_body(rep, c):
        lin_finalize()
        lax.fori_loop(0, NTM, p2_body, 0)
        attn_prologue()
        lax.fori_loop(0, S // TQ, p3_body, 0)

        @pl.when(rep == 0)
        def _():
            lin_reset()
            lax.fori_loop(0, NTM, p4a_body, 0)

        return c

    lax.fori_loop(0, 2, rep_body, 0)
    lax.fori_loop(0, NTM, p4b_body, 0)
    for i in range(NTM):
        out_copy(i).wait()


@jax.jit
def pallas_interleave_layers__linear_attn_block__mha_block__prompt_kernel(
    A_x: jax.Array,
    A_wqkv: jax.Array,
    A_wo: jax.Array,
    B_x: jax.Array,
    B_wqkv: jax.Array,
    B_wo: jax.Array,
):
    del B_x
    x = A_x.reshape(S, D)
    any_spec = pl.BlockSpec(memory_space=pl.ANY)
    out = pl.pallas_call(
        _kernel,
        out_shape=jax.ShapeDtypeStruct((S, D), BF16),
        in_specs=[any_spec] * 5,
        out_specs=any_spec,
        scratch_shapes=[
            pltpu.VMEM((S, D), BF16),
            pltpu.VMEM((D, 3 * D), BF16),
            pltpu.VMEM((D, D), BF16),
            pltpu.VMEM((D, 3 * D), BF16),
            pltpu.VMEM((D, D), BF16),
            pltpu.VMEM((S, D), F32),
            pltpu.VMEM((S, D), BF16),
            pltpu.VMEM((S, D), BF16),
            pltpu.VMEM((S, D), BF16),
            pltpu.VMEM((S // SB, D, SB), BF16),
            pltpu.VMEM((S, D), BF16),
            pltpu.VMEM((G, 128, 128), F32),
            pltpu.VMEM((8, D), F32),
            pltpu.VMEM((G, 128, 256), BF16),
            pltpu.VMEM((LA, KC, 4 * TQ), F32),
            pltpu.SemaphoreType.DMA((NTM,)),
            pltpu.SemaphoreType.DMA((NWCH + 3,)),
            pltpu.SemaphoreType.DMA((NTM,)),
        ],
        compiler_params=pltpu.CompilerParams(vmem_limit_bytes=100 * 1024 * 1024),
    )(x, A_wqkv, A_wo, B_wqkv, B_wo)
    return out.reshape(1, S, D)
```

```python
import functools
import math

import jax
import jax.numpy as jnp
from jax import lax
import jax.experimental.pallas as pl
import jax.experimental.pallas.tpu as pltpu

S = 2048
D = 1024
H = 32
DH = D // H
G = D // 128
SB = 128
NSB = 2
TM = SB * NSB
NTM = S // TM
NC = 256
TQ = 128
NQB = S // TQ
KC = 128
NKC = S // KC
QPI = 1
LA = 2
W_PIECES = [(1024, 256), (1280, 256), (1536, 512), (0, 512), (512, 512)]
NWP = len(W_PIECES)
W_AHEAD = 3
X1_AT = 4

F32 = jnp.float32
BF16 = jnp.bfloat16
Q_SCALE = (DH ** -0.5) * math.log2(math.e)


def _dot(a, b):
    return jnp.dot(a, b, preferred_element_type=F32)


def _dot_nt(a, b):
    return lax.dot_general(a, b, (((1,), (1,)), ((), ())), preferred_element_type=F32)


def _layernorm_bf16(x):
    m = jnp.mean(x, axis=-1, keepdims=True)
    xc = x - m
    v = jnp.mean(xc * xc, axis=-1, keepdims=True)
    return (xc * lax.rsqrt(v + 1e-5)).astype(BF16)


def _phi(t):
    return jnp.where(t > 0, t + 1.0, jnp.exp(t)) + 1e-6


def _rev_rowsum(p):
    n = p.shape[0]
    acc = None
    for t0 in range(0, n, 16):
        for i in range(t0 + 14, t0 - 1, -2):
            t = p[i] + p[i + 1]
            acc = t if acc is None else acc + t
    return acc


def _kernel(x_hbm, wqkva_hbm, woa_hbm, wqkvb_hbm, wob_hbm, out_hbm,
            xio_s, wqkva_s, woa_s, wqkvb_s, wob_s,
            x_s, xn_s, pkt_s, pq_s, q_s, k_s, vt_s, o_s, g_s, z_s, m_s, inv_s, u_s, sc_s, oc_s, lc_s,
            xsem, wsem, osem):

    def x_copy(i):
        rows = pl.ds(pl.multiple_of(i * TM, TM), TM)
        return pltpu.make_async_copy(x_hbm.at[rows, :], xio_s.at[rows, :], xsem.at[i])

    def out_copy(i):
        rows = pl.ds(pl.multiple_of(i * TM, TM), TM)
        return pltpu.make_async_copy(xio_s.at[rows, :], out_hbm.at[rows, :], osem.at[i])

    def wa_copy(j):
        cols = pl.ds(*W_PIECES[j])
        return pltpu.make_async_copy(wqkva_hbm.at[:, cols], wqkva_s.at[:, cols], wsem.at[j])

    vcols = pl.ds(2 * D, D)
    late_copies = [
        pltpu.make_async_copy(wqkva_hbm.at[:, vcols], wqkva_s.at[:, vcols], wsem.at[NWP]),
        pltpu.make_async_copy(woa_hbm, woa_s, wsem.at[NWP + 1]),
        pltpu.make_async_copy(wqkvb_hbm, wqkvb_s, wsem.at[NWP + 2]),
        pltpu.make_async_copy(wob_hbm, wob_s, wsem.at[NWP + 3]),
    ]

    def sub_rows(i, sb):
        return pl.ds(pl.multiple_of(i * TM + sb * SB, SB), SB)

    def lin_post(i, sb, r, c0):
        if c0 < D:
            pq_s[sub_rows(i, sb), c0:c0 + NC] = _phi(r).astype(BF16)
        else:
            pk = _phi(r)
            cz = c0 - D
            z_s[:, cz:cz + NC] += jnp.sum(pk.reshape(SB // 8, 8, NC), axis=0)
            for u in range(NC // 128):
                pkt_s[cz + u * 128:cz + (u + 1) * 128, sb * SB:(sb + 1) * SB] = (
                    pk[:, u * 128:(u + 1) * 128].T.astype(BF16))

    def lin_chunk(i, sb, c0):
        lin_post(i, sb, _dot(xn_s[sb * SB:(sb + 1) * SB, :], wqkva_s[:, c0:c0 + NC]), c0)

    def lin_g():
        for g in range(G):
            a = pkt_s[g * 128:(g + 1) * 128, :]
            for ct in range(G):
                g_s[g, ct] += _dot(a, xn_s[:, ct * 128:(ct + 1) * 128])

    def lin_pass1(i, get_xn):
        for sb in range(NSB):
            xn = get_xn(sb)
            if xn is not None:
                xn_s[sb * SB:(sb + 1) * SB, :] = xn
            for c0 in range(D, 2 * D, NC):
                lin_chunk(i, sb, c0)
        for sb in range(NSB):
            if sb == NSB - 1:
                lin_g()
            for c0 in range(0, D, NC):
                lin_chunk(i, sb, c0)

    def lin_u(i, sb):
        rows = sub_rows(i, sb)
        inv = inv_s[i * NSB + sb]
        parts = []
        for g in range(G):
            bt = jnp.concatenate(
                [jnp.broadcast_to(inv[4 * g + j:4 * g + j + 1, :], (DH, SB)) for j in range(4)], axis=0)
            parts.append(pq_s[rows, g * 128:(g + 1) * 128].astype(F32) * bt.T)
        return jnp.concatenate(parts, axis=1).astype(BF16)

    def lin_finalize(reset):
        r = lax.broadcasted_iota(jnp.int32, (128, 128), 0) // DH
        c = lax.broadcasted_iota(jnp.int32, (128, 128), 1) // DH
        same = r == c
        z = jnp.sum(z_s[...], axis=0, keepdims=True)
        hrow = lax.broadcasted_iota(jnp.int32, (H, D), 0)
        hcol = lax.broadcasted_iota(jnp.int32, (H, D), 1) // DH
        zt = jnp.where(hrow == hcol, jnp.broadcast_to(z, (H, D)), 0.0).astype(BF16)
        nblk = S // SB

        def kv_masked(g):
            gr = slice(g * 128, (g + 1) * 128)
            gg = jnp.concatenate([g_s[g, ct] for ct in range(G)], axis=1)
            kv = _dot(gg.astype(BF16), wqkva_s[:, 2 * D + g * 128:2 * D + (g + 1) * 128])
            if reset:
                g_s[g] = jnp.zeros((G, 128, 128), F32)
            return jnp.where(same, kv, 0.0).astype(BF16)

        kvm = kv_masked(0)
        for g in range(G):
            kvm_next = kv_masked(g + 1) if g + 1 < G else None
            for c0 in range(0, D, 512):
                b = g * (nblk // G) + c0 // 512
                den = _dot_nt(zt, pq_s[b * SB:(b + 1) * SB, :])
                inv_s[b] = 1.0 / (den + 1e-6)
                m_s[g * 128:(g + 1) * 128, c0:c0 + 512] = _dot(
                    kvm, woa_s[g * 128:(g + 1) * 128, c0:c0 + 512]).astype(BF16)
            kvm = kvm_next
        if reset:
            z_s[...] = jnp.zeros(z_s.shape, F32)
        u_s[...] = lin_u(0, 0)

    def out_proj(rows, a, w_ref, src=x_s):
        parts = []
        for c0 in range(0, D, NC):
            xn = src[rows, c0:c0 + NC].astype(F32) + _dot(a, w_ref[:, c0:c0 + NC])
            x_s[rows, c0:c0 + NC] = xn
            parts.append(xn)
        return jnp.concatenate(parts, axis=1)

    def in_ln(i, sb):
        return _layernorm_bf16(xio_s[sub_rows(i, sb), :].astype(F32))

    def p1_first():
        order = [("x", 0)] + [("w", j) for j in range(NWP)]
        order.insert(1 + X1_AT, ("x", 1))
        pos = [0]

        def start_next():
            if pos[0] < len(order):
                kind, j = order[pos[0]]
                (x_copy(j) if kind == "x" else wa_copy(j)).start()
                pos[0] += 1

        for _ in range(W_AHEAD):
            start_next()
        g_s[...] = jnp.zeros(g_s.shape, F32)
        z_s[...] = jnp.zeros(z_s.shape, F32)
        x_copy(0).wait()
        start_next()
        for sb in range(NSB):
            xn_s[sb * SB:(sb + 1) * SB, :] = in_ln(0, sb)
        deferred = []
        for j, (p0, pw) in enumerate(W_PIECES):
            if j == X1_AT:
                x_copy(1).wait()
                start_next()
            wa_copy(j).wait()
            start_next()
            if j == NWP - 1:
                for i in range(2, NTM):
                    x_copy(i).start()
            for args in deferred:
                lin_post(*args)
            deferred = []
            work = [(sb, c0) for sb in range(NSB) for c0 in range(p0, p0 + pw, NC)]
            for n, (sb, c0) in enumerate(work):
                if p0 == 0 and n == len(work) - 1:
                    lin_g()
                r = _dot(xn_s[sb * SB:(sb + 1) * SB, :], wqkva_s[:, c0:c0 + NC])
                if n == len(work) - 1 and j < NWP - 1:
                    deferred.append((0, sb, r, c0))
                else:
                    lin_post(0, sb, r, c0)
        u_s[...] = in_ln(1, 0)

    def p1_body(i, c):
        @pl.when(i + 1 < NTM)
        def _():
            x_copy(i + 1).wait()

        @pl.when(i == 1)
        def _():
            for cp in late_copies:
                cp.start()

        lin_pass1(i, lambda sb: u_s[...] if sb == 0 else in_ln(i, sb))
        u_s[...] = in_ln(jnp.minimum(i + 1, NTM - 1), 0)
        return c

    def p2_body(src, i, c):
        os_ = [u_s[...]] + [lin_u(i, sb) for sb in range(1, NSB)]
        xs = [out_proj(sub_rows(i, sb), os_[sb], m_s, src) for sb in range(NSB)]
        for sb in range(NSB):
            rows = sub_rows(i, sb)
            xn = _layernorm_bf16(xs[sb])
            for c0 in list(range(2 * D, 3 * D, NC)) + list(range(0, 2 * D, NC)):
                r = _dot(xn, wqkvb_s[:, c0:c0 + NC])
                if c0 < D:
                    q_s[rows, c0:c0 + NC] = (r * Q_SCALE).astype(BF16)
                elif c0 < 2 * D:
                    k_s[rows, c0 - D:c0 - D + NC] = r.astype(BF16)
                else:
                    cz = c0 - 2 * D
                    blk = i * NSB + sb
                    for u in range(NC // 128):
                        vt_s[blk, cz + u * 128:cz + (u + 1) * 128, :] = (
                            r[:, u * 128:(u + 1) * 128].T.astype(BF16))
        u_s[...] = lin_u(jnp.minimum(i + 1, NTM - 1), 0)
        return c

    lane_head = lax.broadcasted_iota(jnp.int32, (TQ, 128), 1) // DH

    def q_rows(qb):
        return pl.ds(pl.multiple_of(qb * TQ, TQ), TQ)

    def make_qz(qb, g):
        qf = q_s[q_rows(qb), g * 128:(g + 1) * 128].astype(F32)
        parts = [jnp.where(lane_head == j, qf, 0.0) for j in range(4)]
        return jnp.concatenate(parts, axis=0).astype(BF16)

    def qk_chunk(qz, g, c):
        return _dot_nt(k_s[c * KC:(c + 1) * KC, g * 128:(g + 1) * 128], qz)

    def attn_store(qb, g, oacc, lacc):
        inv = 1.0 / jnp.sum(lacc, axis=0, keepdims=True)
        ot = jnp.concatenate(
            [oacc[j] * inv[:, j * TQ:(j + 1) * TQ] for j in range(4)], axis=0)
        o_s[q_rows(qb), g * 128:(g + 1) * 128] = ot.T.astype(BF16)

    def attn_store_carried(qb):
        attn_store(qb, G - 1, [oc_s[j] for j in range(4)], lc_s[...])

    def attn_prologue():
        qz = make_qz(0, 0)
        for c in range(LA):
            sc_s[c] = qk_chunk(qz, 0, c)
        oc_s[...] = jnp.zeros(oc_s.shape, F32)
        lc_s[...] = jnp.ones(lc_s.shape, F32)

    def p3_body(it, carry):
        N = 4 * TQ
        NST = QPI * G
        qb0 = it * QPI
        attn_store_carried(jnp.maximum(qb0 - 1, 0))
        qb_next = jnp.minimum(qb0 + QPI, NQB - 1)
        qzs = [make_qz(qb0 + st // G, st % G) for st in range(NST)] + [make_qz(qb_next, 0)]
        pend = {c: sc_s[c] for c in range(LA)}
        for st in range(NST):
            g = st % G
            m = None
            lacc = None
            oacc = [None] * 4
            for c in range(NKC):
                t = st * NKC + c
                tn = t + LA
                sn = qk_chunk(qzs[tn // NKC], (tn // NKC) % G, tn % NKC)
                if tn >= NST * NKC:
                    sc_s[tn - NST * NKC] = sn
                else:
                    pend[tn] = sn
                s = pend.pop(t).reshape(KC // 8, 8, N)
                mx = jnp.max(s, axis=0)
                if m is not None:
                    mx = jnp.maximum(mx, m)
                mnew = jnp.broadcast_to(jnp.max(mx, axis=0, keepdims=True), (8, N))
                p = jnp.exp2(s - mnew[None])
                ls = _rev_rowsum(p)
                if m is not None:
                    alpha = jnp.exp2(m - mnew)
                    lacc = lacc * alpha + ls
                else:
                    lacc = ls
                p = p.reshape(KC, N)
                for j in range(4):
                    r0 = g * 128 + j * DH
                    vt = vt_s[c, r0:r0 + DH, :]
                    r = _dot(vt, p[:, j * TQ:(j + 1) * TQ].astype(BF16))
                    if m is None:
                        oacc[j] = r
                    else:
                        a = alpha[:, j * TQ:(j + 1) * TQ]
                        oacc[j] = (oacc[j].reshape(DH // 8, 8, TQ) * a[None]).reshape(DH, TQ) + r
                m = mnew
            if st < NST - 1:
                attn_store(qb0 + st // G, g, oacc, lacc)
            else:
                for j in range(4):
                    oc_s[j] = oacc[j]
                lc_s[...] = lacc
        return carry

    def p4a_body(i, c):
        xs = [out_proj(sub_rows(i, sb), o_s[sub_rows(i, sb), :], wob_s) for sb in range(NSB)]
        lin_pass1(i, lambda sb: _layernorm_bf16(xs[sb]))
        return c

    def p4b_body(i, c):
        for sb in range(NSB):
            rows = sub_rows(i, sb)
            a = o_s[rows, :]
            for c0 in range(0, D, NC):
                xio_s[rows, c0:c0 + NC] = (
                    x_s[rows, c0:c0 + NC] + _dot(a, wob_s[:, c0:c0 + NC])).astype(BF16)
        out_copy(i).start()
        return c

    p1_first()
    lax.fori_loop(1, NTM, p1_body, 0)
    for cp in late_copies:
        cp.wait()
    for rep in range(2):
        lin_finalize(reset=(rep == 0))
        lax.fori_loop(0, NTM, functools.partial(p2_body, xio_s if rep == 0 else x_s), 0)
        attn_prologue()
        lax.fori_loop(0, NQB // QPI, p3_body, 0)
        attn_store_carried(NQB - 1)
        if rep == 0:
            lax.fori_loop(0, NTM, p4a_body, 0)
    lax.fori_loop(0, NTM, p4b_body, 0)
    for i in range(NTM):
        out_copy(i).wait()


@jax.jit
def pallas_interleave_layers__linear_attn_block__mha_block__prompt_kernel(
    A_x: jax.Array,
    A_wqkv: jax.Array,
    A_wo: jax.Array,
    B_x: jax.Array,
    B_wqkv: jax.Array,
    B_wo: jax.Array,
):
    del B_x
    x = A_x.reshape(S, D)
    any_spec = pl.BlockSpec(memory_space=pl.ANY)
    out = pl.pallas_call(
        _kernel,
        out_shape=jax.ShapeDtypeStruct((S, D), BF16),
        in_specs=[any_spec] * 5,
        out_specs=any_spec,
        scratch_shapes=[
            pltpu.VMEM((S, D), BF16),
            pltpu.VMEM((D, 3 * D), BF16),
            pltpu.VMEM((D, D), BF16),
            pltpu.VMEM((D, 3 * D), BF16),
            pltpu.VMEM((D, D), BF16),
            pltpu.VMEM((S, D), F32),
            pltpu.VMEM((TM, D), BF16),
            pltpu.VMEM((D, TM), BF16),
            pltpu.VMEM((S, D), BF16),
            pltpu.VMEM((S, D), BF16),
            pltpu.VMEM((S, D), BF16),
            pltpu.VMEM((S // SB, D, SB), BF16),
            pltpu.VMEM((S, D), BF16),
            pltpu.VMEM((G, G, 128, 128), F32),
            pltpu.VMEM((8, D), F32),
            pltpu.VMEM((D, D), BF16),
            pltpu.VMEM((S // SB, H, SB), F32),
            pltpu.VMEM((SB, D), BF16),
            pltpu.VMEM((LA, KC, 4 * TQ), F32),
            pltpu.VMEM((4, DH, TQ), F32),
            pltpu.VMEM((8, 4 * TQ), F32),
            pltpu.SemaphoreType.DMA((NTM,)),
            pltpu.SemaphoreType.DMA((NWP + 4,)),
            pltpu.SemaphoreType.DMA((NTM,)),
        ],
        compiler_params=pltpu.CompilerParams(vmem_limit_bytes=100 * 1024 * 1024),
    )(x, A_wqkv, A_wo, B_wqkv, B_wo)
    return out.reshape(1, S, D)
```

```python
import functools
import math

import jax
import jax.numpy as jnp
from jax import lax
import jax.experimental.pallas as pl
import jax.experimental.pallas.tpu as pltpu

S = 2048
D = 1024
H = 32
DH = D // H
G = D // 128
SB = 128
NSB = 2
TM = SB * NSB
NTM = S // TM
NC = 256
TQ = 128
NQB = S // TQ
KC = 128
NKC = S // KC
LC = 4
LA = 2
W_PIECES = [(1024, 256), (1280, 256), (1536, 512), (0, 512), (512, 512)]
NWP = len(W_PIECES)
W_AHEAD = 3
X1_AT = 4

F32 = jnp.float32
BF16 = jnp.bfloat16
U32 = jnp.uint32
Q_SCALE = (DH ** -0.5) * math.log2(math.e)


def _dot(a, b):
    return jnp.dot(a, b, preferred_element_type=F32)


def _dot_nt(a, b):
    return lax.dot_general(a, b, (((1,), (1,)), ((), ())), preferred_element_type=F32)


def _pk(x):
    return pltpu.bitcast(x, U32)


def _up(x):
    return pltpu.bitcast(x, BF16)


def _layernorm_bf16(x):
    m = jnp.mean(x, axis=-1, keepdims=True)
    xc = x - m
    v = jnp.mean(xc * xc, axis=-1, keepdims=True)
    return (xc * lax.rsqrt(v + 1e-5)).astype(BF16)


def _phi(t):
    return jnp.where(t > 0, t + 1.0, jnp.exp(t)) + 1e-6


def _rev_rowsum(p):
    n = p.shape[0]
    acc = None
    for t0 in range(0, n, 16):
        for i in range(t0 + 14, t0 - 1, -2):
            t = p[i] + p[i + 1]
            acc = t if acc is None else acc + t
    return acc


def _kernel(x_hbm, wqkva_hbm, woa_hbm, wqkvb_hbm, wob_hbm, out_hbm,
            xio_s, wqkva_s, woa_s, wqkvb_s, wob_s,
            x_s, xn_s, pkt_s, pq_s, qt_s, k_s, vt_s, o_s, g_s, z_s, m_s, inv_s, u_s, sc_s,
            xsem, wsem, osem):

    def x_copy(i):
        rows = pl.ds(pl.multiple_of(i * TM, TM), TM)
        return pltpu.make_async_copy(x_hbm.at[rows, :], xio_s.at[rows, :], xsem.at[i])

    def out_copy(i):
        rows = pl.ds(pl.multiple_of(i * TQ, TQ), TQ)
        return pltpu.make_async_copy(xio_s.at[rows, :], out_hbm.at[rows, :], osem.at[i])

    def wa_copy(j):
        cols = pl.ds(*W_PIECES[j])
        return pltpu.make_async_copy(wqkva_hbm.at[:, cols], wqkva_s.at[:, cols], wsem.at[j])

    vcols = pl.ds(2 * D, D)
    late_copies = [
        pltpu.make_async_copy(wqkva_hbm.at[:, vcols], wqkva_s.at[:, vcols], wsem.at[NWP]),
        pltpu.make_async_copy(woa_hbm, woa_s, wsem.at[NWP + 1]),
        pltpu.make_async_copy(wqkvb_hbm, wqkvb_s, wsem.at[NWP + 2]),
        pltpu.make_async_copy(wob_hbm, wob_s, wsem.at[NWP + 3]),
    ]

    def sub_rows(i, sb):
        return pl.ds(pl.multiple_of(i * TM + sb * SB, SB), SB)

    HB = SB // 2

    def half_rows(blk):
        return pl.ds(pl.multiple_of(blk * HB, HB), HB)

    def lin_post(blk, sb, r, c0):
        if c0 < D:
            pq_s[half_rows(blk), c0:c0 + NC] = _pk(_phi(r).astype(BF16))
        else:
            pk = _phi(r)
            cz = c0 - D
            z_s[:, cz:cz + NC] += jnp.sum(pk.reshape(SB // 8, 8, NC), axis=0)
            for u in range(NC // 128):
                h0 = (cz + u * 128) // 2
                pkt_s[h0:h0 + 64, sb * SB:(sb + 1) * SB] = _pk(
                    pk[:, u * 128:(u + 1) * 128].T.astype(BF16))

    def lin_chunk(blk, sb, c0):
        lin_post(blk, sb, _dot(_up(xn_s[sb * HB:(sb + 1) * HB, :]), wqkva_s[:, c0:c0 + NC]), c0)

    def lin_g(ntok):
        for g in range(G):
            a = _up(pkt_s[g * 64:(g + 1) * 64, 0:ntok])
            for ct in range(G):
                g_s[g, ct] += _dot(a, _up(xn_s[0:ntok // 2, ct * 128:(ct + 1) * 128]))

    def lin_pass1(i, get_xn):
        for sb in range(NSB):
            xn_s[sb * HB:(sb + 1) * HB, :] = get_xn(sb)
            for c0 in range(D, 2 * D, NC):
                lin_chunk(i * NSB + sb, sb, c0)
        for sb in range(NSB):
            if sb == NSB - 1:
                lin_g(TM)
            for c0 in range(0, D, NC):
                lin_chunk(i * NSB + sb, sb, c0)

    def lin_u(i, sb):
        rows = half_rows(i * NSB + sb)
        inv = inv_s[i * NSB + sb]
        parts = []
        for g in range(G):
            bt = jnp.concatenate(
                [jnp.broadcast_to(inv[4 * g + j:4 * g + j + 1, :], (DH, SB)) for j in range(4)], axis=0)
            parts.append(_up(pq_s[rows, g * 128:(g + 1) * 128]).astype(F32) * bt.T)
        return jnp.concatenate(parts, axis=1).astype(BF16)

    def lin_finalize(reset):
        r = lax.broadcasted_iota(jnp.int32, (128, 128), 0) // DH
        c = lax.broadcasted_iota(jnp.int32, (128, 128), 1) // DH
        same = r == c
        z = jnp.sum(z_s[...], axis=0, keepdims=True)
        hrow = lax.broadcasted_iota(jnp.int32, (H, D), 0)
        hcol = lax.broadcasted_iota(jnp.int32, (H, D), 1) // DH
        zt = jnp.where(hrow == hcol, jnp.broadcast_to(z, (H, D)), 0.0).astype(BF16)
        nblk = S // SB

        def kv_masked(g):
            gr = slice(g * 128, (g + 1) * 128)
            gg = jnp.concatenate([g_s[g, ct] for ct in range(G)], axis=1)
            kv = _dot(gg.astype(BF16), wqkva_s[:, 2 * D + g * 128:2 * D + (g + 1) * 128])
            if reset:
                g_s[g] = jnp.zeros((G, 128, 128), F32)
            return jnp.where(same, kv, 0.0).astype(BF16)

        kvm = kv_masked(0)
        for g in range(G):
            kvm_next = kv_masked(g + 1) if g + 1 < G else None
            for c0 in range(0, D, 512):
                b = g * (nblk // G) + c0 // 512
                den = _dot_nt(zt, _up(pq_s[b * HB:(b + 1) * HB, :]))
                inv_s[b] = 1.0 / (den + 1e-6)
                m_s[g * 64:(g + 1) * 64, c0:c0 + 512] = _pk(_dot(
                    kvm, woa_s[g * 128:(g + 1) * 128, c0:c0 + 512]).astype(BF16))
            kvm = kvm_next
        if reset:
            z_s[...] = jnp.zeros(z_s.shape, F32)
        u_s[...] = _pk(lin_u(0, 0))

    def out_proj(rows, a, w_ref, src=x_s):
        parts = []
        for c0 in range(0, D, NC):
            xn = src[rows, c0:c0 + NC].astype(F32) + _dot(a, _up(m_s[:, c0:c0 + NC]) if w_ref is m_s else w_ref[:, c0:c0 + NC])
            x_s[rows, c0:c0 + NC] = xn
            parts.append(xn)
        return jnp.concatenate(parts, axis=1)

    def in_ln(i, sb):
        return _layernorm_bf16(xio_s[sub_rows(i, sb), :].astype(F32))

    def p1_first():
        order = [("x", 0)] + [("w", j) for j in range(NWP)]
        order.insert(1 + X1_AT, ("x", 1))
        pos = [0]

        def start_next():
            if pos[0] < len(order):
                kind, j = order[pos[0]]
                (x_copy(j) if kind == "x" else wa_copy(j)).start()
                pos[0] += 1

        for _ in range(W_AHEAD):
            start_next()
        g_s[...] = jnp.zeros(g_s.shape, F32)
        z_s[...] = jnp.zeros(z_s.shape, F32)
        x_copy(0).wait()
        start_next()
        for sb in range(NSB):
            xn_s[sb * HB:(sb + 1) * HB, :] = _pk(in_ln(0, sb))
        deferred = []
        for j, (p0, pw) in enumerate(W_PIECES):
            if j == X1_AT:
                x_copy(1).wait()
                start_next()
            wa_copy(j).wait()
            start_next()
            if j == NWP - 1:
                for i in range(2, NTM):
                    x_copy(i).start()
            for args in deferred:
                lin_post(*args)
            deferred = []
            work = [(sb, c0) for sb in range(NSB) for c0 in range(p0, p0 + pw, NC)]
            for n, (sb, c0) in enumerate(work):
                if p0 == 0 and n == len(work) - 1:
                    lin_g(TM)
                r = _dot(_up(xn_s[sb * HB:(sb + 1) * HB, :]), wqkva_s[:, c0:c0 + NC])
                if n == len(work) - 1 and j < NWP - 1:
                    deferred.append((sb, sb, r, c0))
                else:
                    lin_post(sb, sb, r, c0)
        u_s[...] = _pk(in_ln(1, 0))

    def p1_body(i, c):
        @pl.when(i + 1 < NTM)
        def _():
            x_copy(i + 1).wait()

        @pl.when(i == 1)
        def _():
            for cp in late_copies:
                cp.start()

        lin_pass1(i, lambda sb: u_s[...] if sb == 0 else _pk(in_ln(i, sb)))
        u_s[...] = _pk(in_ln(jnp.minimum(i + 1, NTM - 1), 0))
        return c

    def p2_body(src, i, c):
        os_ = [_up(u_s[...])] + [lin_u(i, sb) for sb in range(1, NSB)]
        xs = [out_proj(sub_rows(i, sb), os_[sb], m_s, src) for sb in range(NSB)]
        for sb in range(NSB):
            rows = sub_rows(i, sb)
            xn = _layernorm_bf16(xs[sb])
            for c0 in list(range(2 * D, 3 * D, NC)) + list(range(0, 2 * D, NC)):
                r = _dot(xn, wqkvb_s[:, c0:c0 + NC])
                if D <= c0 < 2 * D:
                    k_s[half_rows(i * NSB + sb), c0 - D:c0 - D + NC] = _pk(r.astype(BF16))
                else:
                    dst, cz = (qt_s, c0) if c0 < D else (vt_s, c0 - 2 * D)
                    if c0 < D:
                        r = r * Q_SCALE
                    for u in range(NC // 128):
                        h0 = (cz + u * 128) // 2
                        dst[i * NSB + sb, h0:h0 + 64, :] = _pk(
                            r[:, u * 128:(u + 1) * 128].T.astype(BF16))
        u_s[...] = _pk(lin_u(jnp.minimum(i + 1, NTM - 1), 0))
        return c

    def q_rows(qb):
        return pl.ds(pl.multiple_of(qb * TQ, TQ), TQ)

    def make_qz(qb, g):
        cols = []
        for j in range(4):
            r0 = g * 128 + j * DH
            parts = []
            if j > 0:
                parts.append(jnp.zeros((j * DH, TQ), BF16))
            parts.append(_up(qt_s[qb, r0 // 2:(r0 + DH) // 2, :]))
            if j < 3:
                parts.append(jnp.zeros(((3 - j) * DH, TQ), BF16))
            cols.append(jnp.concatenate(parts, axis=0))
        return jnp.concatenate(cols, axis=1)

    def qk_chunk(qz, g, c):
        return _dot(_up(k_s[c * KC // 2:(c + 1) * KC // 2, g * 128:(g + 1) * 128]), qz)

    def attn_store(g, oacc, lacc):
        inv = 1.0 / jnp.sum(lacc, axis=0, keepdims=True)
        ot = jnp.concatenate(
            [oacc[j] * inv[:, j * TQ:(j + 1) * TQ] for j in range(4)], axis=0)
        o_s[:, g * 128:(g + 1) * 128] = _pk(ot.T.astype(BF16))

    def attn_prologue(ncarry):
        qz = make_qz(0, 0)
        for c in range(ncarry):
            sc_s[c] = qk_chunk(qz, 0, c)

    def p3_body(last, qb, carry):
        N = 4 * TQ
        NT = G * NKC
        ncarry = LA if last else LC
        rows = q_rows(qb)
        qzs = [make_qz(qb, g) for g in range(G)]
        pend = {c: sc_s[c] for c in range(ncarry)}
        nxt = [ncarry]
        KA = (G - 1) * 128

        def part_a(n):
            c0 = n * NC
            x_s[rows, c0:c0 + NC] += _dot(_up(o_s[:, 0:KA]), wob_s[0:KA, c0:c0 + NC])

        nfill = 0
        for g in range(G):
            m = None
            lacc = None
            oacc = [None] * 4
            for c in range(NKC):
                t = g * NKC + c
                tn = nxt[0]
                if tn < NT:
                    if tn - t <= LA or t % 2 == 0:
                        pend[tn] = qk_chunk(qzs[tn // NKC], tn // NKC, tn % NKC)
                        nxt[0] += 1
                else:
                    part_a(nfill)
                    nfill += 1
                s = pend.pop(t).reshape(KC // 8, 8, N)
                mx = jnp.max(s, axis=0)
                if m is not None:
                    mx = jnp.maximum(mx, m)
                mnew = jnp.broadcast_to(jnp.max(mx, axis=0, keepdims=True), (8, N))
                p = jnp.exp2(s - mnew[None])
                ls = _rev_rowsum(p)
                if m is not None:
                    alpha = jnp.exp2(m - mnew)
                    lacc = lacc * alpha + ls
                else:
                    lacc = ls
                p = p.reshape(KC, N)
                for j in range(4):
                    r0 = g * 128 + j * DH
                    vt = _up(vt_s[c, r0 // 2:(r0 + DH) // 2, :])
                    r = _dot(vt, p[:, j * TQ:(j + 1) * TQ].astype(BF16))
                    if m is None:
                        oacc[j] = r
                    else:
                        a = alpha[:, j * TQ:(j + 1) * TQ]
                        oacc[j] = (oacc[j].reshape(DH // 8, 8, TQ) * a[None]).reshape(DH, TQ) + r
                m = mnew
            attn_store(g, oacc, lacc)
        for n in range(nfill, D // NC):
            part_a(n)

        def lookahead():
            qz = make_qz(jnp.minimum(qb + 1, NQB - 1), 0)
            for c in range(ncarry):
                sc_s[c] = qk_chunk(qz, 0, c)

        def part_b(c0):
            return x_s[rows, c0:c0 + NC] + _dot(_up(o_s[:, KA:D]), wob_s[KA:D, c0:c0 + NC])

        if last:
            lookahead()
            for c0 in range(0, D, NC):
                xio_s[rows, c0:c0 + NC] = part_b(c0).astype(BF16)
            out_copy(qb).start()
        else:
            parts = []
            for c0 in range(0, D, NC):
                xn = part_b(c0)
                x_s[rows, c0:c0 + NC] = xn
                parts.append(xn)
            lookahead()
            xn_s[0:HB, :] = _pk(_layernorm_bf16(jnp.concatenate(parts, axis=1)))
            for c0 in list(range(D, 2 * D, NC)) + list(range(0, D // 2, NC)):
                lin_chunk(qb, 0, c0)
            lin_g(SB)
            for c0 in range(D // 2, D, NC):
                lin_chunk(qb, 0, c0)
        return carry

    p1_first()
    lax.fori_loop(1, NTM, p1_body, 0)
    for cp in late_copies:
        cp.wait()
    for rep in range(2):
        last = rep == 1
        lin_finalize(reset=not last)
        lax.fori_loop(0, NTM, functools.partial(p2_body, x_s if last else xio_s), 0)
        attn_prologue(LA if last else LC)
        lax.fori_loop(0, NQB, functools.partial(p3_body, last), 0)
    for i in range(NQB):
        out_copy(i).wait()


@jax.jit
def pallas_interleave_layers__linear_attn_block__mha_block__prompt_kernel(
    A_x: jax.Array,
    A_wqkv: jax.Array,
    A_wo: jax.Array,
    B_x: jax.Array,
    B_wqkv: jax.Array,
    B_wo: jax.Array,
):
    del B_x
    x = A_x.reshape(S, D)
    any_spec = pl.BlockSpec(memory_space=pl.ANY)
    out = pl.pallas_call(
        _kernel,
        out_shape=jax.ShapeDtypeStruct((S, D), BF16),
        in_specs=[any_spec] * 5,
        out_specs=any_spec,
        scratch_shapes=[
            pltpu.VMEM((S, D), BF16),
            pltpu.VMEM((D, 3 * D), BF16),
            pltpu.VMEM((D, D), BF16),
            pltpu.VMEM((D, 3 * D), BF16),
            pltpu.VMEM((D, D), BF16),
            pltpu.VMEM((S, D), F32),
            pltpu.VMEM((TM // 2, D), U32),
            pltpu.VMEM((D // 2, TM), U32),
            pltpu.VMEM((S // 2, D), U32),
            pltpu.VMEM((S // SB, D // 2, SB), U32),
            pltpu.VMEM((S // 2, D), U32),
            pltpu.VMEM((S // SB, D // 2, SB), U32),
            pltpu.VMEM((TQ // 2, D), U32),
            pltpu.VMEM((G, G, 128, 128), F32),
            pltpu.VMEM((8, D), F32),
            pltpu.VMEM((D // 2, D), U32),
            pltpu.VMEM((S // SB, H, SB), F32),
            pltpu.VMEM((SB // 2, D), U32),
            pltpu.VMEM((LC, KC, 4 * TQ), F32),
            pltpu.SemaphoreType.DMA((NTM,)),
            pltpu.SemaphoreType.DMA((NWP + 4,)),
            pltpu.SemaphoreType.DMA((NQB,)),
        ],
        compiler_params=pltpu.CompilerParams(vmem_limit_bytes=100 * 1024 * 1024),
    )(x, A_wqkv, A_wo, B_wqkv, B_wo)
    return out.reshape(1, S, D)
```

```python
import functools
import math

import jax
import jax.numpy as jnp
from jax import lax
import jax.experimental.pallas as pl
import jax.experimental.pallas.tpu as pltpu

S = 2048
D = 1024
H = 32
DH = D // H
G = D // 128
SB = 128
NSB = 2
TM = SB * NSB
NTM = S // TM
NC = 256
TQ = 128
NQB = S // TQ
KC = 128
NKC = S // KC
LC = 4
LA = 2
W_PIECES = [(1024, 256), (1280, 256), (1536, 512), (0, 512), (512, 512)]
NWP = len(W_PIECES)
EARLY1 = 1

F32 = jnp.float32
BF16 = jnp.bfloat16
U32 = jnp.uint32
Q_SCALE = (DH ** -0.5) * math.log2(math.e)


def _dot(a, b):
    return jnp.dot(a, b, preferred_element_type=F32)


def _dot_nt(a, b):
    return lax.dot_general(a, b, (((1,), (1,)), ((), ())), preferred_element_type=F32)


def _pk(x):
    return pltpu.bitcast(x, U32)


def _up(x):
    return pltpu.bitcast(x, BF16)


def _layernorm_bf16(x):
    m = jnp.mean(x, axis=-1, keepdims=True)
    xc = x - m
    v = jnp.mean(xc * xc, axis=-1, keepdims=True)
    return (xc * lax.rsqrt(v + 1e-5)).astype(BF16)


def _phi(t):
    return jnp.where(t > 0, t + 1.0, jnp.exp(t)) + 1e-6


def _rev_rowsum(p):
    n = p.shape[0]
    acc = None
    for t0 in range(0, n, 16):
        for i in range(t0 + 14, t0 - 1, -2):
            t = p[i] + p[i + 1]
            acc = t if acc is None else acc + t
    return acc


def _kernel(x_hbm, wqkva_hbm, woa_hbm, wqkvb_hbm, wob_hbm, out_hbm,
            xio_s, wqkva_s, woa_s, wqkvb_s, wob_s,
            x_s, xn_s, pkt_s, pq_s, qt_s, k_s, vt_s, o_s, g_s, z_s, m_s, inv_s, u_s, sc_s,
            xsem, wsem, osem):

    def x_copy(i):
        rows = pl.ds(pl.multiple_of(i * TM, TM), TM)
        return pltpu.make_async_copy(x_hbm.at[rows, :], xio_s.at[rows, :], xsem.at[i])

    def out_copy(i):
        rows = pl.ds(pl.multiple_of(i * TQ, TQ), TQ)
        return pltpu.make_async_copy(xio_s.at[rows, :], out_hbm.at[rows, :], osem.at[0])

    def wa_copy(j):
        cols = pl.ds(*W_PIECES[j])
        return pltpu.make_async_copy(wqkva_hbm.at[:, cols], wqkva_s.at[:, cols], wsem.at[j])

    vcols = pl.ds(2 * D, D)
    late_copies = [
        pltpu.make_async_copy(wqkva_hbm.at[:, vcols], wqkva_s.at[:, vcols], wsem.at[NWP]),
        pltpu.make_async_copy(woa_hbm, woa_s, wsem.at[NWP]),
        pltpu.make_async_copy(wqkvb_hbm, wqkvb_s, wsem.at[NWP]),
        pltpu.make_async_copy(wob_hbm, wob_s, wsem.at[NWP]),
    ]

    def sub_rows(i, sb):
        return pl.ds(pl.multiple_of(i * TM + sb * SB, SB), SB)

    HB = SB // 2

    def half_rows(blk):
        return pl.ds(pl.multiple_of(blk * HB, HB), HB)

    def lin_post(blk, sb, r, c0):
        if c0 < D:
            pq_s[half_rows(blk), c0:c0 + NC] = _pk(_phi(r).astype(BF16))
        else:
            pk = _phi(r)
            cz = c0 - D
            z_s[:, cz:cz + NC] += jnp.sum(pk.reshape(SB // 8, 8, NC), axis=0)
            for u in range(NC // 128):
                h0 = (cz + u * 128) // 2
                pkt_s[h0:h0 + 64, sb * SB:(sb + 1) * SB] = _pk(
                    pk[:, u * 128:(u + 1) * 128].T.astype(BF16))

    def lin_chunk(blk, sb, c0):
        lin_post(blk, sb, _dot(_up(xn_s[sb * HB:(sb + 1) * HB, :]), wqkva_s[:, c0:c0 + NC]), c0)

    def lin_g(ntok, groups=range(G)):
        for g in groups:
            a = _up(pkt_s[g * 64:(g + 1) * 64, 0:ntok])
            for ct in range(G):
                g_s[g, ct] += _dot(a, _up(xn_s[0:ntok // 2, ct * 128:(ct + 1) * 128]))

    def lin_pass1(i, get_xn):
        for sb in range(NSB):
            xn_s[sb * HB:(sb + 1) * HB, :] = get_xn(sb)
            for c0 in range(D, 2 * D, NC):
                lin_chunk(i * NSB + sb, sb, c0)
        for sb in range(NSB):
            if sb == NSB - 1:
                lin_g(TM)
            for c0 in range(0, D, NC):
                lin_chunk(i * NSB + sb, sb, c0)

    def lin_u(i, sb):
        rows = half_rows(i * NSB + sb)
        inv = inv_s[i * NSB + sb]
        parts = []
        for g in range(G):
            bt = jnp.concatenate(
                [jnp.broadcast_to(inv[4 * g + j:4 * g + j + 1, :], (DH, SB)) for j in range(4)], axis=0)
            parts.append(_up(pq_s[rows, g * 128:(g + 1) * 128]).astype(F32) * bt.T)
        return jnp.concatenate(parts, axis=1).astype(BF16)

    def lin_finalize(reset):
        r = lax.broadcasted_iota(jnp.int32, (128, 128), 0) // DH
        c = lax.broadcasted_iota(jnp.int32, (128, 128), 1) // DH
        same = r == c
        z = jnp.sum(z_s[...], axis=0, keepdims=True)
        hrow = lax.broadcasted_iota(jnp.int32, (H, D), 0)
        hcol = lax.broadcasted_iota(jnp.int32, (H, D), 1) // DH
        zt = jnp.where(hrow == hcol, jnp.broadcast_to(z, (H, D)), 0.0).astype(BF16)
        nblk = S // SB

        def kv_masked(g):
            gr = slice(g * 128, (g + 1) * 128)
            gg = jnp.concatenate([g_s[g, ct] for ct in range(G)], axis=1)
            kv = _dot(gg.astype(BF16), wqkva_s[:, 2 * D + g * 128:2 * D + (g + 1) * 128])
            if reset:
                g_s[g] = jnp.zeros((G, 128, 128), F32)
            return jnp.where(same, kv, 0.0).astype(BF16)

        kvm = kv_masked(0)
        for g in range(G):
            kvm_next = kv_masked(g + 1) if g + 1 < G else None
            for c0 in range(0, D, 512):
                b = g * (nblk // G) + c0 // 512
                den = _dot_nt(zt, _up(pq_s[b * HB:(b + 1) * HB, :]))
                inv_s[b] = 1.0 / (den + 1e-6)
                m_s[g * 64:(g + 1) * 64, c0:c0 + 512] = _pk(_dot(
                    kvm, woa_s[g * 128:(g + 1) * 128, c0:c0 + 512]).astype(BF16))
            kvm = kvm_next
        if reset:
            z_s[...] = jnp.zeros(z_s.shape, F32)
        u_s[...] = _pk(lin_u(0, 0))

    def out_proj(rows, a, w_ref, src=x_s):
        parts = []
        for c0 in range(0, D, NC):
            xn = src[rows, c0:c0 + NC].astype(F32) + _dot(a, _up(m_s[:, c0:c0 + NC]) if w_ref is m_s else w_ref[:, c0:c0 + NC])
            x_s[rows, c0:c0 + NC] = xn
            parts.append(xn)
        return jnp.concatenate(parts, axis=1)

    def in_ln(i, sb):
        return _layernorm_bf16(xio_s[sub_rows(i, sb), :].astype(F32))

    def p1_first():
        def x0_copy(sb):
            rows = pl.ds(sb * SB, SB)
            return pltpu.make_async_copy(x_hbm.at[rows, :], xio_s.at[rows, :], osem.at[sb])

        x0_copy(0).start()
        wa_copy(0).start()
        for sb in range(1, NSB):
            x0_copy(sb).start()
        g_s[...] = jnp.zeros(g_s.shape, F32)
        z_s[...] = jnp.zeros(z_s.shape, F32)
        x0_copy(0).wait()
        if EARLY1:
            wa_copy(1).start()
        xn_s[0:HB, :] = _pk(in_ln(0, 0))
        deferred = []
        gdone = 0
        for j, (p0, pw) in enumerate(W_PIECES):
            wa_copy(j).wait()
            if j == 0:
                for sb in range(1, NSB):
                    x0_copy(sb).wait()
                if not EARLY1:
                    wa_copy(1).start()
            if j + 2 < NWP:
                wa_copy(j + 2).start()
            if j == NWP - 2:
                x_copy(1).start()
            if j == NWP - 1:
                x_copy(1).wait()
                for i in range(2, NTM):
                    x_copy(i).start()
            if j == 0:
                for sb in range(1, NSB):
                    xn_s[sb * HB:(sb + 1) * HB, :] = _pk(in_ln(0, sb))
            for args in deferred:
                lin_post(*args)
            deferred = []
            for c0 in range(p0, p0 + pw, NC):
                gready = (c0 - D) // 128 if c0 >= D else G
                for sb in range(NSB):
                    r = _dot(_up(xn_s[sb * HB:(sb + 1) * HB, :]), wqkva_s[:, c0:c0 + NC])
                    if (sb == NSB - 1 and c0 + NC == p0 + pw and j < NWP - 1
                            and gready == gdone):
                        deferred.append((sb, sb, r, c0))
                    else:
                        lin_post(sb, sb, r, c0)
                lin_g(TM, range(gdone, gready))
                gdone = gready
        u_s[...] = _pk(in_ln(1, 0))

    def p1_body(i, c):
        @pl.when(i + 1 < NTM)
        def _():
            x_copy(i + 1).wait()

        @pl.when(i == 1)
        def _():
            for cp in late_copies:
                cp.start()

        lin_pass1(i, lambda sb: u_s[...] if sb == 0 else _pk(in_ln(i, sb)))
        u_s[...] = _pk(in_ln(jnp.minimum(i + 1, NTM - 1), 0))
        return c

    def p2_body(src, i, c):
        os_ = [_up(u_s[...])] + [lin_u(i, sb) for sb in range(1, NSB)]
        xs = [out_proj(sub_rows(i, sb), os_[sb], m_s, src) for sb in range(NSB)]
        for sb in range(NSB):
            rows = sub_rows(i, sb)
            xn = _layernorm_bf16(xs[sb])
            for c0 in list(range(2 * D, 3 * D, NC)) + list(range(0, 2 * D, NC)):
                r = _dot(xn, wqkvb_s[:, c0:c0 + NC])
                if D <= c0 < 2 * D:
                    k_s[half_rows(i * NSB + sb), c0 - D:c0 - D + NC] = _pk(r.astype(BF16))
                else:
                    dst, cz = (qt_s, c0) if c0 < D else (vt_s, c0 - 2 * D)
                    if c0 < D:
                        r = r * Q_SCALE
                    for u in range(NC // 128):
                        h0 = (cz + u * 128) // 2
                        dst[i * NSB + sb, h0:h0 + 64, :] = _pk(
                            r[:, u * 128:(u + 1) * 128].T.astype(BF16))
        u_s[...] = _pk(lin_u(jnp.minimum(i + 1, NTM - 1), 0))
        return c

    def q_rows(qb):
        return pl.ds(pl.multiple_of(qb * TQ, TQ), TQ)

    def make_qz(qb, g):
        cols = []
        for j in range(4):
            r0 = g * 128 + j * DH
            parts = []
            if j > 0:
                parts.append(jnp.zeros((j * DH, TQ), BF16))
            parts.append(_up(qt_s[qb, r0 // 2:(r0 + DH) // 2, :]))
            if j < 3:
                parts.append(jnp.zeros(((3 - j) * DH, TQ), BF16))
            cols.append(jnp.concatenate(parts, axis=0))
        return jnp.concatenate(cols, axis=1)

    def qk_chunk(qz, g, c):
        return _dot(_up(k_s[c * KC // 2:(c + 1) * KC // 2, g * 128:(g + 1) * 128]), qz)

    def attn_store(g, oacc, lacc):
        inv = 1.0 / jnp.sum(lacc, axis=0, keepdims=True)
        ot = jnp.concatenate(
            [oacc[j] * inv[:, j * TQ:(j + 1) * TQ] for j in range(4)], axis=0)
        o_s[:, g * 128:(g + 1) * 128] = _pk(ot.T.astype(BF16))

    def attn_prologue(ncarry):
        qz = make_qz(0, 0)
        for c in range(ncarry):
            sc_s[c] = qk_chunk(qz, 0, c)

    def p3_body(last, qb, carry):
        N = 4 * TQ
        NT = G * NKC
        ncarry = 0 if last else LC
        rows = q_rows(qb)
        qzs = [make_qz(qb, g) for g in range(G)]
        pend = {c: sc_s[c] for c in range(ncarry)}
        nxt = [ncarry]
        KA = (G - 1) * 128

        def part_a(n):
            c0 = n * NC
            x_s[rows, c0:c0 + NC] += _dot(_up(o_s[:, 0:KA]), wob_s[0:KA, c0:c0 + NC])

        nfill = 0
        for g in range(G):
            m = None
            lacc = None
            oacc = [None] * 4
            for c in range(NKC):
                t = g * NKC + c
                while t == 0 and nxt[0] < LA:
                    pend[nxt[0]] = qk_chunk(qzs[0], 0, nxt[0])
                    nxt[0] += 1
                tn = nxt[0]
                if tn < NT:
                    if tn - t <= LA or t % 2 == 0:
                        pend[tn] = qk_chunk(qzs[tn // NKC], tn // NKC, tn % NKC)
                        nxt[0] += 1
                else:
                    part_a(nfill)
                    nfill += 1
                s = pend.pop(t).reshape(KC // 8, 8, N)
                mx = jnp.max(s, axis=0)
                if m is not None:
                    mx = jnp.maximum(mx, m)
                mnew = jnp.broadcast_to(jnp.max(mx, axis=0, keepdims=True), (8, N))
                p = jnp.exp2(s - mnew[None])
                ls = _rev_rowsum(p)
                if m is not None:
                    alpha = jnp.exp2(m - mnew)
                    lacc = lacc * alpha + ls
                else:
                    lacc = ls
                p = p.reshape(KC, N)
                for j in range(4):
                    r0 = g * 128 + j * DH
                    vt = _up(vt_s[c, r0 // 2:(r0 + DH) // 2, :])
                    r = _dot(vt, p[:, j * TQ:(j + 1) * TQ].astype(BF16))
                    if m is None:
                        oacc[j] = r
                    else:
                        a = alpha[:, j * TQ:(j + 1) * TQ]
                        oacc[j] = (oacc[j].reshape(DH // 8, 8, TQ) * a[None]).reshape(DH, TQ) + r
                m = mnew
            attn_store(g, oacc, lacc)
        for n in range(nfill, D // NC):
            part_a(n)

        def lookahead():
            qz = make_qz(jnp.minimum(qb + 1, NQB - 1), 0)
            for c in range(ncarry):
                sc_s[c] = qk_chunk(qz, 0, c)

        def part_b(c0):
            return x_s[rows, c0:c0 + NC] + _dot(_up(o_s[:, KA:D]), wob_s[KA:D, c0:c0 + NC])

        if last:
            for c0 in range(0, D, NC):
                xio_s[rows, c0:c0 + NC] = part_b(c0).astype(BF16)
            out_copy(qb).start()
        else:
            parts = []
            for c0 in range(0, D, NC):
                xn = part_b(c0)
                x_s[rows, c0:c0 + NC] = xn
                parts.append(xn)
            lookahead()
            xn_s[0:HB, :] = _pk(_layernorm_bf16(jnp.concatenate(parts, axis=1)))
            for c0 in list(range(D, 2 * D, NC)) + list(range(0, D // 2, NC)):
                lin_chunk(qb, 0, c0)
            lin_g(SB)
            for c0 in range(D // 2, D, NC):
                lin_chunk(qb, 0, c0)
        return carry

    p1_first()
    lax.fori_loop(1, NTM, p1_body, 0)
    for cp in late_copies:
        cp.wait()
    for rep in range(2):
        last = rep == 1
        lin_finalize(reset=not last)
        lax.fori_loop(0, NTM, functools.partial(p2_body, x_s if last else xio_s), 0)
        if not last:
            attn_prologue(LC)
        lax.fori_loop(0, NQB, functools.partial(p3_body, last), 0)
    for i in range(NQB):
        out_copy(i).wait()


@jax.jit
def pallas_interleave_layers__linear_attn_block__mha_block__prompt_kernel(
    A_x: jax.Array,
    A_wqkv: jax.Array,
    A_wo: jax.Array,
    B_x: jax.Array,
    B_wqkv: jax.Array,
    B_wo: jax.Array,
):
    del B_x
    x = A_x.reshape(S, D)
    any_spec = pl.BlockSpec(memory_space=pl.ANY)
    out = pl.pallas_call(
        _kernel,
        out_shape=jax.ShapeDtypeStruct((S, D), BF16),
        in_specs=[any_spec] * 5,
        out_specs=any_spec,
        scratch_shapes=[
            pltpu.VMEM((S, D), BF16),
            pltpu.VMEM((D, 3 * D), BF16),
            pltpu.VMEM((D, D), BF16),
            pltpu.VMEM((D, 3 * D), BF16),
            pltpu.VMEM((D, D), BF16),
            pltpu.VMEM((S, D), F32),
            pltpu.VMEM((TM // 2, D), U32),
            pltpu.VMEM((D // 2, TM), U32),
            pltpu.VMEM((S // 2, D), U32),
            pltpu.VMEM((S // SB, D // 2, SB), U32),
            pltpu.VMEM((S // 2, D), U32),
            pltpu.VMEM((S // SB, D // 2, SB), U32),
            pltpu.VMEM((TQ // 2, D), U32),
            pltpu.VMEM((G, G, 128, 128), F32),
            pltpu.VMEM((8, D), F32),
            pltpu.VMEM((D // 2, D), U32),
            pltpu.VMEM((S // SB, H, SB), F32),
            pltpu.VMEM((SB // 2, D), U32),
            pltpu.VMEM((LC, KC, 4 * TQ), F32),
            pltpu.SemaphoreType.DMA((NTM,)),
            pltpu.SemaphoreType.DMA((NWP + 1,)),
            pltpu.SemaphoreType.DMA((NSB,)),
        ],
        compiler_params=pltpu.CompilerParams(vmem_limit_bytes=100 * 1024 * 1024),
    )(x, A_wqkv, A_wo, B_wqkv, B_wo)
    return out.reshape(1, S, D)
```

```python
import functools
import math

import jax
import jax.numpy as jnp
from jax import lax
import jax.experimental.pallas as pl
import jax.experimental.pallas.tpu as pltpu

S = 2048
D = 1024
H = 32
DH = D // H
G = D // 128
SB = 128
NSB = 2
TM = SB * NSB
NTM = S // TM
NC = 256
TQ = 128
NQB = S // TQ
KC = 128
NKC = S // KC
LA = 2
LC = 4
W_PIECES = [(1024, 256), (1280, 256), (1536, 512), (0, 512), (512, 512)]
NWP = len(W_PIECES)

F32 = jnp.float32
BF16 = jnp.bfloat16
U32 = jnp.uint32
Q_SCALE = (DH ** -0.5) * math.log2(math.e)


def _dot(a, b):
    return jnp.dot(a, b, preferred_element_type=F32)


def _dot_nt(a, b):
    return lax.dot_general(a, b, (((1,), (1,)), ((), ())), preferred_element_type=F32)


def _pk(x):
    return pltpu.bitcast(x, U32)


def _up(x):
    return pltpu.bitcast(x, BF16)


def _layernorm_bf16(x):
    m = jnp.mean(x, axis=-1, keepdims=True)
    xc = x - m
    v = jnp.mean(xc * xc, axis=-1, keepdims=True)
    return (xc * lax.rsqrt(v + 1e-5)).astype(BF16)


def _phi(t):
    return jnp.where(t > 0, t + 1.0, jnp.exp(t)) + 1e-6


def _rev_rowsum(p):
    n = p.shape[0]
    acc = None
    for t0 in range(0, n, 16):
        for i in range(t0 + 14, t0 - 1, -2):
            t = p[i] + p[i + 1]
            acc = t if acc is None else acc + t
    return acc


def _kernel(x_hbm, wqkva_hbm, woa_hbm, wqkvb_hbm, wob_hbm, out_hbm,
            xio_s, wqkva_s, woa_s, wqkvb_s, wob_s,
            x_s, xn_s, pkt_s, pq_s, qt_s, k_s, vt_s, o_s, g_s, z_s, m_s, inv_s, u_s, sc_s,
            xsem, wsem, osem):

    def x_copy(i):
        rows = pl.ds(pl.multiple_of(i * TM, TM), TM)
        return pltpu.make_async_copy(x_hbm.at[rows, :], xio_s.at[rows, :], xsem.at[i])

    def out_copy(i):
        rows = pl.ds(pl.multiple_of(i * TQ, TQ), TQ)
        return pltpu.make_async_copy(xio_s.at[rows, :], out_hbm.at[rows, :], osem.at[0])

    def wa_copy(j):
        cols = pl.ds(*W_PIECES[j])
        return pltpu.make_async_copy(wqkva_hbm.at[:, cols], wqkva_s.at[:, cols], wsem.at[j])

    vcols = pl.ds(2 * D, D)
    late_copies = [
        pltpu.make_async_copy(wqkva_hbm.at[:, vcols], wqkva_s.at[:, vcols], wsem.at[NWP]),
        pltpu.make_async_copy(woa_hbm, woa_s, wsem.at[NWP]),
        pltpu.make_async_copy(wqkvb_hbm, wqkvb_s, wsem.at[NWP]),
        pltpu.make_async_copy(wob_hbm, wob_s, wsem.at[NWP]),
    ]

    def sub_rows(i, sb):
        return pl.ds(pl.multiple_of(i * TM + sb * SB, SB), SB)

    HB = SB // 2

    def half_rows(blk):
        return pl.ds(pl.multiple_of(blk * HB, HB), HB)

    def lin_post(blk, sb, r, c0):
        if c0 < D:
            pq_s[half_rows(blk), c0:c0 + NC] = _pk(_phi(r).astype(BF16))
        else:
            pk = _phi(r)
            cz = c0 - D
            z_s[:, cz:cz + NC] += jnp.sum(pk.reshape(SB // 8, 8, NC), axis=0)
            for u in range(NC // 128):
                h0 = (cz + u * 128) // 2
                pkt_s[h0:h0 + 64, sb * SB:(sb + 1) * SB] = _pk(
                    pk[:, u * 128:(u + 1) * 128].T.astype(BF16))

    def lin_chunk(blk, sb, c0):
        lin_post(blk, sb, _dot(_up(xn_s[sb * HB:(sb + 1) * HB, :]), wqkva_s[:, c0:c0 + NC]), c0)

    def lin_g(ntok, groups=range(G)):
        for g in groups:
            a = _up(pkt_s[g * 64:(g + 1) * 64, 0:ntok])
            for ct in range(G):
                g_s[g, ct] += _dot(a, _up(xn_s[0:ntok // 2, ct * 128:(ct + 1) * 128]))

    def lin_pass1(i, get_xn):
        for sb in range(NSB):
            xn_s[sb * HB:(sb + 1) * HB, :] = get_xn(sb)
            for c0 in range(D, 2 * D, NC):
                lin_chunk(i * NSB + sb, sb, c0)
        for sb in range(NSB):
            for c0 in range(0, D, NC):
                lin_chunk(i * NSB + sb, sb, c0)
        lin_g(TM)

    def lin_u(i, sb):
        rows = half_rows(i * NSB + sb)
        inv = inv_s[i * NSB + sb]
        parts = []
        for g in range(G):
            bt = jnp.concatenate(
                [jnp.broadcast_to(inv[4 * g + j:4 * g + j + 1, :], (DH, SB)) for j in range(4)], axis=0)
            parts.append(_up(pq_s[rows, g * 128:(g + 1) * 128]).astype(F32) * bt.T)
        return jnp.concatenate(parts, axis=1).astype(BF16)

    def lin_finalize(reset):
        r = lax.broadcasted_iota(jnp.int32, (128, 128), 0) // DH
        c = lax.broadcasted_iota(jnp.int32, (128, 128), 1) // DH
        same = r == c
        z = jnp.sum(z_s[...], axis=0, keepdims=True)
        hrow = lax.broadcasted_iota(jnp.int32, (H, D), 0)
        hcol = lax.broadcasted_iota(jnp.int32, (H, D), 1) // DH
        zt = jnp.where(hrow == hcol, jnp.broadcast_to(z, (H, D)), 0.0).astype(BF16)
        nblk = S // SB

        def kv_masked(g):
            gg = jnp.concatenate([g_s[g, ct] for ct in range(G)], axis=1)
            kv = _dot(gg.astype(BF16), wqkva_s[:, 2 * D + g * 128:2 * D + (g + 1) * 128])
            if reset:
                g_s[g] = jnp.zeros((G, 128, 128), F32)
            return jnp.where(same, kv, 0.0).astype(BF16)

        kvm = kv_masked(0)
        for g in range(G):
            kvm_next = kv_masked(g + 1) if g + 1 < G else None
            for c0 in range(0, D, 512):
                b = g * (nblk // G) + c0 // 512
                den = _dot_nt(zt, _up(pq_s[b * HB:(b + 1) * HB, :]))
                inv_s[b] = 1.0 / (den + 1e-6)
                m_s[g * 64:(g + 1) * 64, c0:c0 + 512] = _pk(_dot(
                    kvm, woa_s[g * 128:(g + 1) * 128, c0:c0 + 512]).astype(BF16))
            kvm = kvm_next
        if reset:
            z_s[...] = jnp.zeros(z_s.shape, F32)
        u_s[...] = _pk(lin_u(0, 0))

    def lin_out(rows, u, src):
        parts = []
        for c0 in range(0, D, NC):
            xn = src[rows, c0:c0 + NC].astype(F32) + _dot(u, _up(m_s[:, c0:c0 + NC]))
            x_s[rows, c0:c0 + NC] = xn
            parts.append(xn)
        return jnp.concatenate(parts, axis=1)

    def in_ln(i, sb):
        return _layernorm_bf16(xio_s[sub_rows(i, sb), :].astype(F32))

    def p1_first():
        def x0_copy(sb):
            rows = pl.ds(sb * SB, SB)
            return pltpu.make_async_copy(x_hbm.at[rows, :], xio_s.at[rows, :], osem.at[sb])

        x0_copy(0).start()
        wa_copy(0).start()
        for sb in range(1, NSB):
            x0_copy(sb).start()
        g_s[...] = jnp.zeros(g_s.shape, F32)
        z_s[...] = jnp.zeros(z_s.shape, F32)
        x0_copy(0).wait()
        wa_copy(1).start()
        xn_s[0:HB, :] = _pk(in_ln(0, 0))
        deferred = []
        gdone = 0
        for j, (p0, pw) in enumerate(W_PIECES):
            wa_copy(j).wait()
            if j == 0:
                for sb in range(1, NSB):
                    x0_copy(sb).wait()
            if j + 2 < NWP:
                wa_copy(j + 2).start()
            if j == NWP - 2:
                x_copy(1).start()
            if j == NWP - 1:
                x_copy(1).wait()
                for i in range(2, NTM):
                    x_copy(i).start()
            if j == 0:
                for sb in range(1, NSB):
                    xn_s[sb * HB:(sb + 1) * HB, :] = _pk(in_ln(0, sb))
            for args in deferred:
                lin_post(*args)
            deferred = []
            for c0 in range(p0, p0 + pw, NC):
                gready = (c0 - D) // 128 if c0 >= D else G
                for sb in range(NSB):
                    r = _dot(_up(xn_s[sb * HB:(sb + 1) * HB, :]), wqkva_s[:, c0:c0 + NC])
                    if (sb == NSB - 1 and c0 + NC == p0 + pw and j < NWP - 1
                            and gready == gdone):
                        deferred.append((sb, sb, r, c0))
                    else:
                        lin_post(sb, sb, r, c0)
                lin_g(TM, range(gdone, gready))
                gdone = gready
        u_s[...] = _pk(in_ln(1, 0))

    def p1_body(i, c):
        @pl.when(i + 1 < NTM)
        def _():
            x_copy(i + 1).wait()

        @pl.when(i == 1)
        def _():
            for cp in late_copies:
                cp.start()

        lin_pass1(i, lambda sb: u_s[...] if sb == 0 else _pk(in_ln(i, sb)))
        u_s[...] = _pk(in_ln(jnp.minimum(i + 1, NTM - 1), 0))
        return c

    def p2_body(src, i, c):
        us = [_up(u_s[...])] + [lin_u(i, sb) for sb in range(1, NSB)]
        xs = [lin_out(sub_rows(i, sb), us[sb], src) for sb in range(NSB)]
        for sb in range(NSB):
            xn = _layernorm_bf16(xs[sb])
            for c0 in list(range(2 * D, 3 * D, NC)) + list(range(0, 2 * D, NC)):
                r = _dot(xn, wqkvb_s[:, c0:c0 + NC])
                if D <= c0 < 2 * D:
                    k_s[half_rows(i * NSB + sb), c0 - D:c0 - D + NC] = _pk(r.astype(BF16))
                else:
                    dst, cz = (qt_s, c0) if c0 < D else (vt_s, c0 - 2 * D)
                    if c0 < D:
                        r = r * Q_SCALE
                    for u in range(NC // 128):
                        h0 = (cz + u * 128) // 2
                        dst[i * NSB + sb, h0:h0 + 64, :] = _pk(
                            r[:, u * 128:(u + 1) * 128].T.astype(BF16))
        u_s[...] = _pk(lin_u(jnp.minimum(i + 1, NTM - 1), 0))
        return c

    def q_rows(qb):
        return pl.ds(pl.multiple_of(qb * TQ, TQ), TQ)

    def make_qz(qb, g):
        cols = []
        for j in range(4):
            r0 = g * 128 + j * DH
            parts = []
            if j > 0:
                parts.append(jnp.zeros((j * DH, TQ), BF16))
            parts.append(_up(qt_s[qb, r0 // 2:(r0 + DH) // 2, :]))
            if j < 3:
                parts.append(jnp.zeros(((3 - j) * DH, TQ), BF16))
            cols.append(jnp.concatenate(parts, axis=0))
        return jnp.concatenate(cols, axis=1)

    def qk_chunk(qz, g, c):
        return _dot(_up(k_s[c * KC // 2:(c + 1) * KC // 2, g * 128:(g + 1) * 128]), qz)

    def attn_store(g, oacc, lacc):
        inv = 1.0 / jnp.sum(lacc, axis=0, keepdims=True)
        ot = jnp.concatenate(
            [oacc[j] * inv[:, j * TQ:(j + 1) * TQ] for j in range(4)], axis=0)
        o_s[:, g * 128:(g + 1) * 128] = _pk(ot.T.astype(BF16))

    def attn_prologue(ncarry):
        qz = make_qz(0, 0)
        for c in range(ncarry):
            sc_s[c] = qk_chunk(qz, 0, c)

    def p3_body(last, qb, carry):
        N = 4 * TQ
        NT = G * NKC
        ncarry = 0 if last else LC
        rows = q_rows(qb)
        qzs = [make_qz(qb, g) for g in range(G)]
        pend = {c: sc_s[c] for c in range(ncarry)}
        nxt = [ncarry]
        KA = (G - 1) * 128

        def part_a(n):
            c0 = n * NC
            x_s[rows, c0:c0 + NC] += _dot(_up(o_s[:, 0:KA]), wob_s[0:KA, c0:c0 + NC])

        nfill = 0
        for g in range(G):
            m = None
            lacc = None
            oacc = [None] * 4
            for c in range(NKC):
                t = g * NKC + c
                while t == 0 and nxt[0] < LA:
                    pend[nxt[0]] = qk_chunk(qzs[0], 0, nxt[0])
                    nxt[0] += 1
                tn = nxt[0]
                if tn < NT:
                    if tn - t <= LA or t % 2 == 0:
                        pend[tn] = qk_chunk(qzs[tn // NKC], tn // NKC, tn % NKC)
                        nxt[0] += 1
                else:
                    part_a(nfill)
                    nfill += 1
                s = pend.pop(t).reshape(KC // 8, 8, N)
                mx = jnp.max(s, axis=0)
                if m is not None:
                    mx = jnp.maximum(mx, m)
                mnew = jnp.broadcast_to(jnp.max(mx, axis=0, keepdims=True), (8, N))
                p = jnp.exp2(s - mnew[None])
                ls = _rev_rowsum(p)
                if m is not None:
                    alpha = jnp.exp2(m - mnew)
                    lacc = lacc * alpha + ls
                else:
                    lacc = ls
                p = p.reshape(KC, N)
                for j in range(4):
                    r0 = g * 128 + j * DH
                    vt = _up(vt_s[c, r0 // 2:(r0 + DH) // 2, :])
                    r = _dot(vt, p[:, j * TQ:(j + 1) * TQ].astype(BF16))
                    if m is None:
                        oacc[j] = r
                    else:
                        a = alpha[:, j * TQ:(j + 1) * TQ]
                        oacc[j] = (oacc[j].reshape(DH // 8, 8, TQ) * a[None]).reshape(DH, TQ) + r
                m = mnew
            attn_store(g, oacc, lacc)
        for n in range(nfill, D // NC):
            part_a(n)

        def lookahead():
            qz = make_qz(jnp.minimum(qb + 1, NQB - 1), 0)
            for c in range(ncarry):
                sc_s[c] = qk_chunk(qz, 0, c)

        def part_b(c0):
            return x_s[rows, c0:c0 + NC] + _dot(_up(o_s[:, KA:D]), wob_s[KA:D, c0:c0 + NC])

        if last:
            for c0 in range(0, D, NC):
                xio_s[rows, c0:c0 + NC] = part_b(c0).astype(BF16)
            out_copy(qb).start()
        else:
            parts = []
            for c0 in range(0, D, NC):
                xn = part_b(c0)
                x_s[rows, c0:c0 + NC] = xn
                parts.append(xn)
            lookahead()
            xn_s[0:HB, :] = _pk(_layernorm_bf16(jnp.concatenate(parts, axis=1)))
            for c0 in list(range(D, 2 * D, NC)) + list(range(0, D, NC)):
                lin_chunk(qb, 0, c0)
            lin_g(SB)
        return carry

    p1_first()
    lax.fori_loop(1, NTM, p1_body, 0)
    for cp in late_copies:
        cp.wait()
    for rep in range(2):
        last = rep == 1
        lin_finalize(reset=not last)
        lax.fori_loop(0, NTM, functools.partial(p2_body, x_s if last else xio_s), 0)
        if not last:
            attn_prologue(LC)
        lax.fori_loop(0, NQB, functools.partial(p3_body, last), 0)
    for i in range(NQB):
        out_copy(i).wait()


@jax.jit
def pallas_interleave_layers__linear_attn_block__mha_block__prompt_kernel(
    A_x: jax.Array,
    A_wqkv: jax.Array,
    A_wo: jax.Array,
    B_x: jax.Array,
    B_wqkv: jax.Array,
    B_wo: jax.Array,
):
    del B_x
    x = A_x.reshape(S, D)
    any_spec = pl.BlockSpec(memory_space=pl.ANY)
    out = pl.pallas_call(
        _kernel,
        out_shape=jax.ShapeDtypeStruct((S, D), BF16),
        in_specs=[any_spec] * 5,
        out_specs=any_spec,
        scratch_shapes=[
            pltpu.VMEM((S, D), BF16),
            pltpu.VMEM((D, 3 * D), BF16),
            pltpu.VMEM((D, D), BF16),
            pltpu.VMEM((D, 3 * D), BF16),
            pltpu.VMEM((D, D), BF16),
            pltpu.VMEM((S, D), F32),
            pltpu.VMEM((TM // 2, D), U32),
            pltpu.VMEM((D // 2, TM), U32),
            pltpu.VMEM((S // 2, D), U32),
            pltpu.VMEM((S // SB, D // 2, SB), U32),
            pltpu.VMEM((S // 2, D), U32),
            pltpu.VMEM((S // SB, D // 2, SB), U32),
            pltpu.VMEM((TQ // 2, D), U32),
            pltpu.VMEM((G, G, 128, 128), F32),
            pltpu.VMEM((8, D), F32),
            pltpu.VMEM((D // 2, D), U32),
            pltpu.VMEM((S // SB, H, SB), F32),
            pltpu.VMEM((SB // 2, D), U32),
            pltpu.VMEM((LC, KC, 4 * TQ), F32),
            pltpu.SemaphoreType.DMA((NTM,)),
            pltpu.SemaphoreType.DMA((NWP + 1,)),
            pltpu.SemaphoreType.DMA((NSB,)),
        ],
        compiler_params=pltpu.CompilerParams(vmem_limit_bytes=100 * 1024 * 1024),
    )(x, A_wqkv, A_wo, B_wqkv, B_wo)
    return out.reshape(1, S, D)
```
